```python
import jax
import jax.numpy as jnp

def _softmax(x, axis=-1):
    return jax.nn.softmax(x, axis=axis)
def _gelu(x):
    return jax.nn.gelu(x, approximate=True)
def _silu(x):
    return jax.nn.silu(x)
def _sigmoid(x):
    return jax.nn.sigmoid(x)
def _layernorm(x, axis=-1, eps=1e-5):
    m = jnp.mean(x, axis=axis, keepdims=True)
    v = jnp.var(x, axis=axis, keepdims=True)
    return (x - m) / jnp.sqrt(v + eps)
def _scatter_add(tgt, idx, src, axis=0):
    return tgt.at[idx].add(src)
def _segment_sum(src, seg, n):
    return jax.ops.segment_sum(src, seg, n)
class _Rng:
    def __init__(self, key):
        self._k = key
    def _next(self):
        self._k, sub = jax.random.split(self._k)
        return sub
    def normal(self, shape):
        return jax.random.normal(self._next(), shape, dtype=jnp.bfloat16)
    def randint(self, lo, hi, shape):
        return jax.random.randint(self._next(), shape, lo, hi, dtype=jnp.int32)
    def uniform(self, shape, lo=0.0, hi=1.0):
        return jax.random.uniform(self._next(), shape, jnp.bfloat16, lo, hi)
    def permutation(self, n):
        return jax.random.permutation(self._next(), n)


kernel_name = 'interleave_layers__sliding_block_cached__dense_activation_gelu__decode'

def setup_inputs():
    _rng = _Rng(jax.random.key(int.from_bytes(__import__("os").urandom(4), "little")))
    _w = (lambda a: (lambda t: t.astype(jnp.bfloat16) if jnp.issubdtype(t.dtype, jnp.floating) else t)(jnp.asarray(a)))
    def _A_setup():
        B, Sq, D = 1, 1, 640
        Hq, Hkv, Sk, Dh = 32, 32, 32768, 192
        assert Hq % Hkv == 0, (Hq, Hkv)
        return {
            "x": _w((lambda *s: _rng.normal(s) * 0.05)(B, Sq, D)),
            "k_cache": _w((lambda *s: _rng.normal(s) * 0.05)(B, Hkv, Sk, Dh)),
            "v_cache": _w((lambda *s: _rng.normal(s) * 0.05)(B, Hkv, Sk, Dh)),
            "wq": _w((lambda *s: _rng.normal(s) * 0.05)(D, Hq * Dh) * (D ** -0.5)),
            "wo": _w((lambda *s: _rng.normal(s) * 0.05)(Hq * Dh, D) * ((Hq * Dh) ** -0.5)),
        }
    _A_in = _A_setup()

    def _B_setup():
        B, S, D, F = 1, 1, 640, 1536
        return {
            "x": _w((lambda *s: _rng.normal(s) * 0.05)(B, S, D)),
            "w1": _w((lambda *s: _rng.normal(s) * 0.05)(D, F) * (D ** -0.5)),
            "b1": _w((lambda *s: _rng.normal(s) * 0.05)(F) * 0.01),
            "w2": _w((lambda *s: _rng.normal(s) * 0.05)(F, D) * (F ** -0.5)),
            "b2": _w((lambda *s: _rng.normal(s) * 0.05)(D) * 0.01),
        }
    _B_in = _B_setup()

    return {
        "A_x": _A_in["x"],
        "A_k_cache": _A_in["k_cache"],
        "A_v_cache": _A_in["v_cache"],
        "A_wq": _A_in["wq"],
        "A_wo": _A_in["wo"],
        "B_x": _B_in["x"],
        "B_w1": _B_in["w1"],
        "B_b1": _B_in["b1"],
        "B_w2": _B_in["w2"],
        "B_b2": _B_in["b2"],
    }

def reference(A_x, A_k_cache, A_v_cache, A_wq, A_wo, B_x, B_w1, B_b1, B_w2, B_b2):
    def _A_ref(x, k_cache, v_cache, wq, wo):
        B, Sq, D = x.shape
        Hq, Dh = 32, 192
        Hkv, Sk = k_cache.shape[1], k_cache.shape[2]
        W = min(4096, max(256, Sk // 4))
        rep = Hq // Hkv
        q = (lambda x, *d: x.transpose(*d))((x @ wq).reshape(B, Sq, Hq, Dh), 0, 2, 1, 3)
        k = jnp.repeat(k_cache[:, :, Sk - W:, :], rep, axis=1)
        v = jnp.repeat(v_cache[:, :, Sk - W:, :], rep, axis=1)
        scores = jnp.einsum("bhqd,bhkd->bhqk", q, k) * (Dh ** -0.5)
        p = _softmax(scores, axis=-1)
        o = jnp.einsum("bhqk,bhkd->bhqd", p, v)
        return (lambda x, *d: x.transpose(*d))(o, 0, 2, 1, 3).reshape(B, Sq, Hq * Dh) @ wo

    def _B_ref(x, w1, b1, w2, b2):
        h = jnp.einsum("bsd,df->bsf", x, w1) + b1
        h = _gelu(h)
        return jnp.einsum("bsf,fd->bsd", h, w2) + b2

    x = A_x
    x = x + _A_ref(_layernorm(x, axis=-1), A_k_cache, A_v_cache, A_wq, A_wo)
    x = x + _B_ref(_layernorm(x, axis=-1), B_w1, B_b1, B_w2, B_b2)
    x = x + _A_ref(_layernorm(x, axis=-1), A_k_cache, A_v_cache, A_wq, A_wo)
    x = x + _B_ref(_layernorm(x, axis=-1), B_w1, B_b1, B_w2, B_b2)
    return x
```

```python
import jax
import jax.numpy as jnp
from jax import lax
import jax.experimental.pallas as pl
import jax.experimental.pallas.tpu as pltpu

H, DH = 32, 192
PAIR = 2 * DH
NP = H // 2
LANES = 128
bf = jnp.bfloat16
f32 = jnp.float32
u32 = jnp.uint32


def _rb(v):
    return v.astype(bf).astype(f32)


def _ln(x):
    m = jnp.mean(x, axis=-1, keepdims=True)
    d = x - m
    v = jnp.mean(d * d, axis=-1, keepdims=True)
    return d / jnp.sqrt(v + 1e-5)


def _tile(ref32, j, r0, n):
    return pltpu.bitcast(ref32[j, pl.ds(r0 // 2 if isinstance(r0, int) else pl.multiple_of(r0 // 2, 32), n // 2), :], bf)


def _cat(ref32, nt, r0, n, base=0):
    return jnp.concatenate([_tile(ref32, base + j, r0, n) for j in range(nt)], axis=1)


def make(SK, W, D, F, GP=4, NL=2, dma=True):
    NS = W // LANES
    NC = NS // 4
    ND = D // LANES
    NF = F // LANES
    NG = NP // GP
    GR = GP * PAIR
    c_exp = (DH ** -0.5) * 1.4426950408889634

    def kern(x_hbm, k_hbm, v_hbm, wq_hbm, wo_hbm, w1_hbm, b1_hbm, w2_hbm, b2_hbm, o_ref,
             kb, vb, wqb, wob, w1b, w2b, xb, b1b, b2b, xn_s, q_s, s_s, p_s, o_s, acc_s, x_s,
             semk, semv, semq, semo, semf, sems):
        kb32, vb32, wq32, wo32, w132, w232 = (r.bitcast(u32) for r in (kb, vb, wqb, wob, w1b, w2b))

        def start_kv(src, dst, sem, g):
            r = pl.ds(g * GR if isinstance(g, int) else pl.multiple_of(g * GR, GR), GR)
            for j in range(NS):
                pltpu.make_async_copy(src.at[r, pl.ds(SK - W + j * LANES, LANES)], dst.at[j, r], sem.at[g]).start()
        def start_w(src, dst, sem):
            for j in range(dst.shape[0]):
                pltpu.make_async_copy(src.at[:, pl.ds(j * LANES, LANES)], dst.at[j], sem).start()
        cx = pltpu.make_async_copy(x_hbm, xb, sems.at[0])
        c1 = pltpu.make_async_copy(b1_hbm, b1b, sems.at[1])
        c2 = pltpu.make_async_copy(b2_hbm, b2b, sems.at[2])
        def wait_group(buf, sem, g):
            t = buf.at[:, pl.ds(0, GR)]
            pltpu.make_async_copy(t, t, sem.at[g]).wait()
        def wait_all(buf, sem):
            pltpu.make_async_copy(buf, buf, sem).wait()

        cx.start()
        if dma:
            start_w(wq_hbm, wqb, semq.at[0])
        c1.start(); c2.start()
        if dma:
            start_kv(k_hbm, kb, semk, 0)
            start_w(wo_hbm, wob, semo.at[0])
        cx.wait(); c1.wait(); c2.wait()
        x_s[...] = jnp.broadcast_to(xb[0].astype(f32), (8, D))
        if dma:
            wait_all(wqb, semq.at[0])
            start_kv(v_hbm, vb, semv, 0)

        row = lax.broadcasted_iota(jnp.int32, (8, 4 * PAIR), 0)
        col = lax.broadcasted_iota(jnp.int32, (8, 4 * PAIR), 1)
        qmask = jnp.logical_and(col >= row * DH, col < (row + 1) * DH)

        def q_proj(i):
            q = jnp.dot(xn_s[...].astype(bf), _cat(wq32, 3, 0, D, base=3 * i), preferred_element_type=f32)
            return jnp.where(qmask, jnp.concatenate([q] * 4, axis=1), 0.0)

        def k_chunk(lhs, i, c):
            rhs = jnp.concatenate([_tile(kb32, 4 * c + t, i * PAIR, PAIR) for t in range(4)], axis=0)
            return jnp.dot(lhs, rhs, preferred_element_type=f32)

        def k_scores(lhs, i):
            return jnp.concatenate([k_chunk(lhs, i, c) for c in range(NC)], axis=1)

        def softmax(s):
            m = jnp.max(s, axis=1, keepdims=True)
            m = jnp.broadcast_to(m, (8, LANES))
            m = jnp.maximum(m, pltpu.roll(m, 2, 0))
            m = jnp.maximum(m, pltpu.roll(m, 4, 0))
            e = jnp.exp2((s - jnp.concatenate([m] * NC, axis=1)) * c_exp)
            l = jnp.sum(e, axis=1, keepdims=True)
            l = jnp.broadcast_to(l, (8, LANES))
            l = l + pltpu.roll(l, 2, 0)
            l = l + pltpu.roll(l, 4, 0)
            return e * jnp.concatenate([1.0 / l] * NC, axis=1)

        def pv_part(acc, i, slot, a, js):
            for j in js:
                c, t = divmod(j, 4)
                p = jnp.broadcast_to(p_s[slot, 2 * t + a:2 * t + a + 1, c * LANES:(c + 1) * LANES], (DH, LANES))
                y = _tile(vb32, j, i * PAIR + a * DH, DH).astype(f32) * p
                acc = y if acc is None else acc + y
            return acc

        def o_proj(o, i):
            return jnp.dot(o.astype(bf), _cat(wo32, ND, i * PAIR, PAIR), preferred_element_type=f32)

        def layer(li, carry):
            first = jnp.logical_and(li == 0, dma)
            xn_s[...] = _ln(x_s[...])
            @pl.when(first)
            def _():
                wait_group(kb, semk, 0)
                start_kv(k_hbm, kb, semk, 1)
            s0 = k_scores(q_proj(0).astype(bf), 0)
            s_s[...] = k_scores(q_proj(1).astype(bf), 1)
            p_s[0] = softmax(s0)
            q_s[...] = q_proj(2)
            o_s[...] = jnp.zeros((8, PAIR), f32)
            acc_s[...] = jnp.zeros((8, D), f32)
            @pl.when(first)
            def _():
                wait_all(wob, semo.at[0])

            def step(i, c_):
                @pl.when(first)
                def _():
                    @pl.when(i % GP == 0)
                    def _():
                        g = i // GP
                        @pl.when(g + 1 < NG)
                        def _():
                            start_kv(v_hbm, vb, semv, g + 1)
                        @pl.when(g + 1 == NG)
                        def _():
                            start_w(w1_hbm, w1b, semf.at[0])
                            start_w(w2_hbm, w2b, semf.at[1])
                        wait_group(vb, semv, g)
                    @pl.when(jnp.logical_and((i + 2) % GP == 0, i + 2 < NP))
                    def _():
                        g = (i + 2) // GP
                        @pl.when(g + 1 < NG)
                        def _():
                            start_kv(k_hbm, kb, semk, g + 1)
                        wait_group(kb, semk, g)
                slot = i % 2
                ik = jnp.minimum(i + 2, NP - 1)
                iq = jnp.minimum(i + 3, NP - 1)
                lhs = q_s[...].astype(bf)
                s_prev = s_s[...]
                o_prev = o_s[...]
                sc = []
                accs = []
                for a in range(2):
                    acc = None
                    for u in range(NC // 2):
                        sc.append(k_chunk(lhs, ik, a * (NC // 2) + u))
                        acc = pv_part(acc, i, slot, a, range(8 * u, 8 * u + 8))
                        if u == 1 and a == 0:
                            acc_s[...] += o_proj(o_prev, jnp.maximum(i - 1, 0))
                        if u == 2 and a == 0:
                            p_s[1 - slot] = softmax(s_prev)
                        if u == 1 and a == 1:
                            q_s[...] = q_proj(iq)
                    accs.append(acc)
                s_s[...] = jnp.concatenate(sc, axis=1)
                acc = jnp.concatenate(accs, axis=0)
                o = jnp.sum(acc.T, axis=0, keepdims=True)
                o_s[...] = jnp.broadcast_to(o, (8, PAIR))
                return c_
            lax.fori_loop(0, NP, step, 0)
            x1 = _rb(x_s[...] + _rb(acc_s[...] + o_proj(o_s[...], NP - 1)))
            @pl.when(first)
            def _():
                wait_all(w1b, semf.at[0])
            h = jnp.dot(_ln(x1).astype(bf), _cat(w132, NF, 0, D), preferred_element_type=f32)
            h = _rb(_rb(h) + b1b[...].astype(f32).reshape(1, F))
            h = jax.nn.gelu(h, approximate=True)
            @pl.when(first)
            def _():
                wait_all(w2b, semf.at[1])
            y = jnp.dot(h.astype(bf), _cat(w232, ND, 0, F), preferred_element_type=f32)
            y = _rb(_rb(y) + b2b[...].astype(f32).reshape(1, D))
            x_s[...] = _rb(x1 + y)
            return carry
        lax.fori_loop(0, NL, layer, 0)
        o_ref[0] = x_s[0:1, :].astype(o_ref.dtype)

    any_ = pl.BlockSpec(memory_space=pl.ANY)
    return pl.pallas_call(
        kern,
        out_shape=jax.ShapeDtypeStruct((1, 1, D), bf),
        in_specs=[any_] * 9,
        scratch_shapes=[
            pltpu.VMEM((NS, H * DH, LANES), bf), pltpu.VMEM((NS, H * DH, LANES), bf),
            pltpu.VMEM((3 * NP, D, LANES), bf), pltpu.VMEM((ND, H * DH, LANES), bf),
            pltpu.VMEM((NF, D, LANES), bf), pltpu.VMEM((ND, F, LANES), bf),
            pltpu.VMEM((1, 1, D), bf), pltpu.VMEM((F,), bf), pltpu.VMEM((D,), bf),
            pltpu.VMEM((8, D), f32), pltpu.VMEM((8, 4 * PAIR), f32), pltpu.VMEM((8, W // 4), f32),
            pltpu.VMEM((2, 8, W // 4), f32), pltpu.VMEM((8, PAIR), f32), pltpu.VMEM((8, D), f32),
            pltpu.VMEM((8, D), f32),
            pltpu.SemaphoreType.DMA((NG,)), pltpu.SemaphoreType.DMA((NG,)), pltpu.SemaphoreType.DMA((1,)),
            pltpu.SemaphoreType.DMA((1,)), pltpu.SemaphoreType.DMA((2,)), pltpu.SemaphoreType.DMA((3,)),
        ],
        compiler_params=pltpu.CompilerParams(vmem_limit_bytes=124 * 1024 * 1024),
        name="fused_layers",
    )


def kernel(A_x, A_k_cache, A_v_cache, A_wq, A_wo, B_x, B_w1, B_b1, B_w2, B_b2, **kw):
    SK = A_k_cache.shape[2]
    W = min(4096, max(256, SK // 4))
    D, F = B_w1.shape
    kt = jnp.swapaxes(A_k_cache, 2, 3).reshape(H * DH, SK)
    vt = jnp.swapaxes(A_v_cache, 2, 3).reshape(H * DH, SK)
    return make(SK, W, D, F, **kw)(A_x, kt, vt, A_wq, A_wo, B_w1, B_b1, B_w2, B_b2)


@jax.jit
def pallas_interleave_layers__sliding_block_cached__dense_activation_gelu__decode_kernel(
    A_x, A_k_cache, A_v_cache, A_wq, A_wo, B_x, B_w1, B_b1, B_w2, B_b2
):
    return kernel(A_x, A_k_cache, A_v_cache, A_wq, A_wo, B_x, B_w1, B_b1, B_w2, B_b2)
```

```python
import jax
import jax.numpy as jnp
from jax import lax
import jax.experimental.pallas as pl
import jax.experimental.pallas.tpu as pltpu

H, DH = 32, 192
PAIR = 2 * DH
NP = H // 2
LANES = 128
bf = jnp.bfloat16
f32 = jnp.float32
u32 = jnp.uint32


def _rb(v):
    return v.astype(bf).astype(f32)


def _ln(x):
    m = jnp.mean(x, axis=-1, keepdims=True)
    d = x - m
    v = jnp.mean(d * d, axis=-1, keepdims=True)
    return d / jnp.sqrt(v + 1e-5)


def _rows32(r0, n):
    h = r0 // 2
    return pl.ds(h if isinstance(h, int) else pl.multiple_of(h, 8), n // 2)


def _tile(ref32, j, r0, n):
    return pltpu.bitcast(ref32[j, _rows32(r0, n), :], bf)


def _cat(ref32, nt, r0, n, base=0):
    return jnp.concatenate([_tile(ref32, base + j, r0, n) for j in range(nt)], axis=1)


def _dot(a, b):
    return lax.dot_general(a, b, (((1,), (0,)), ((), ())), preferred_element_type=f32)


def make(SK, W, D, F, GP=2, NL=2, dma=True, flags=None, NM=10, GRW=32, ORDER='kmqo', T0=4, T1=0, PV=48, AH=2):
    NS = W // LANES
    NC = NS // 4
    ND = D // LANES
    NF = F // LANES
    NG = NP // GP
    GR = GP * PAIR
    c_exp = (DH ** -0.5) * 1.4426950408889634

    def kern(x_hbm, k_hbm, v_hbm, wq_hbm, wo_hbm, w1_hbm, b1_hbm, w2_hbm, b2_hbm, o_ref,
             kb, vb, wqb, wob, w1b, w2b, xb, b1b, b2b, xn_s, q_s, s_s, p_s, a_s, z_s, o_s, acc_s, x_s,
             semk, semv, semq, semo, sem1, sem2, sems):
        kb32, vb32, wq32, wo32, w132, w232 = (r.bitcast(u32) for r in (kb, vb, wqb, wob, w1b, w2b))

        def start_kv(src, dst, sem, g):
            r = pl.ds(g * GR if isinstance(g, int) else pl.multiple_of(g * GR, GR), GR)
            @pl.loop(0, NS)
            def _(j):
                c = pl.ds(pl.multiple_of(SK - W + j * LANES, LANES), LANES)
                pltpu.make_async_copy(src.at[r, c], dst.at[j, r], sem.at[g]).start()

        def start_w(src, dst, sem):
            @pl.loop(0, dst.shape[0])
            def _(j):
                c = pl.ds(pl.multiple_of(j * LANES, LANES), LANES)
                pltpu.make_async_copy(src.at[:, c], dst.at[j], sem).start()

        def wait_group(buf, sem, g):
            t = buf.at[:, pl.ds(0, GR)]
            pltpu.make_async_copy(t, t, sem.at[g]).wait()

        def wait_all(buf, sem):
            pltpu.make_async_copy(buf, buf, sem).wait()

        cx = pltpu.make_async_copy(x_hbm, xb, sems.at[0])
        c1 = pltpu.make_async_copy(b1_hbm, b1b, sems.at[1])
        c2 = pltpu.make_async_copy(b2_hbm, b2b, sems.at[2])
        if dma:
            start_w(wo_hbm, wob, semo.at[0])
        cx.start(); c1.start(); c2.start()
        if dma:
            start_w(wq_hbm, wqb, semq.at[0])
            start_kv(k_hbm, kb, semk, 0)
            start_kv(v_hbm, vb, semv, 0)
        z_s[...] = jnp.zeros((8, LANES), jnp.int32)
        cx.wait(); c1.wait(); c2.wait()
        x_s[...] = jnp.broadcast_to(xb[0].astype(f32), (8, D))
        if dma:
            wait_all(wob, semo.at[0])
            wait_all(wqb, semq.at[0])
            wait_group(kb, semk, 0)

        row = lax.broadcasted_iota(jnp.int32, (8, 4 * PAIR), 0)
        col = lax.broadcasted_iota(jnp.int32, (8, 4 * PAIR), 1)
        qmask = jnp.logical_and(col >= row * DH, col < (row + 1) * DH)
        row1 = lax.broadcasted_iota(jnp.int32, (8, LANES), 0)
        omask = (lax.broadcasted_iota(jnp.int32, (8, PAIR), 0) & 1) == (
            lax.broadcasted_iota(jnp.int32, (8, PAIR), 1) >= DH).astype(jnp.int32)

        def q_proj(i):
            return _dot(xn_s[...], _cat(wq32, 3, 0, D, base=3 * i))

        def q_lhs(q):
            return jnp.where(qmask, jnp.concatenate([_rb(q)] * 4, axis=1), 0.0)

        def k_scores(lhs, i):
            rhs = jnp.concatenate(
                [jnp.concatenate([_tile(kb32, 4 * c + t, i * PAIR, PAIR) for t in range(4)], axis=0)
                 for c in range(NC)], axis=1)
            return _dot(lhs, rhs)

        def softmax(s):
            m = jnp.max(s, axis=1, keepdims=True)
            m = jnp.broadcast_to(m, (8, LANES))
            m = jnp.maximum(m, pltpu.roll(m, 2, 0))
            m = jnp.maximum(m, pltpu.roll(m, 4, 0))
            e = jnp.exp2((s - jnp.concatenate([m] * NC, axis=1)) * c_exp)
            l = jnp.sum(e, axis=1, keepdims=True)
            l = jnp.broadcast_to(l, (8, LANES))
            l = l + pltpu.roll(l, 2, 0)
            l = l + pltpu.roll(l, 4, 0)
            return e, l

        def pv_vpu(i, g, never, tok):
            a = g * GRW // DH
            acc = None
            for j in range(NM, NS):
                c, t = divmod(j, 4)
                p = jnp.broadcast_to(p_s[2 * t + a:2 * t + a + 1, c * LANES:(c + 1) * LANES], (GRW, LANES))
                y = _tile(vb32, j, i * PAIR + g * GRW, GRW).astype(f32) * p
                if acc is None and tok is not None:
                    y = jnp.where(never, jnp.concatenate([tok] * (GRW // 8), axis=0), y)
                acc = y if acc is None else acc + y
            return acc

        def pv_mxu(i, e):
            lhs = jnp.concatenate([jnp.where((row1 >> 1) == j % 4, e[:, (j // 4) * LANES:(j // 4 + 1) * LANES], 0.0)
                                   for j in range(NM)], axis=1)
            rhs = jnp.concatenate(
                [jnp.concatenate([_tile(vb32, j, i * PAIR + n * LANES, LANES) for j in range(NM)], axis=0)
                 for n in range(3)], axis=1)
            return _dot(lhs, rhs)

        def o_red():
            o = jnp.sum(jnp.concatenate([a_s[...].T, o_s[0]], axis=0), axis=0, keepdims=True)
            l = jnp.sum(o_s[1], axis=0, keepdims=True)
            return jnp.broadcast_to(o / l, (8, PAIR))

        def o_proj(o, i):
            return _dot(o, _cat(wo32, ND, i * PAIR, PAIR))

        def layer(li, carry):
            first = jnp.logical_and(li == 0, dma)
            xn_s[...] = _ln(x_s[...])
            s_s[...] = k_scores(q_lhs(q_proj(0)), 0)
            q_s[...] = q_lhs(q_proj(1))
            o_s[0] = jnp.zeros((8, PAIR), f32)
            o_s[1] = jnp.ones((8, PAIR), f32)
            a_s[...] = jnp.zeros((PAIR, LANES), f32)
            acc_s[...] = jnp.zeros((8, D), f32)

            def fetch(i, last):
                @pl.when(i % GP == 0)
                def _():
                    g = i // GP
                    @pl.when(g + 1 < NG)
                    def _():
                        start_kv(k_hbm, kb, semk, g + 1)
                    @pl.when(g + 1 == NG)
                    def _():
                        start_w(w1_hbm, w1b, sem1.at[0])
                        start_w(w2_hbm, w2b, sem2.at[0])
                    wait_group(vb, semv, g)
                @pl.loop(0, NM // AH)
                def _(j):
                    ts = [[pltpu.bitcast(_tile(vb32, j * AH + m, i * PAIR + n * LANES, LANES).T, u32) for n in range(3)] for m in range(AH)]
                    for m in range(AH):
                        vb32[j * AH + m, _rows32(i * PAIR, PAIR), :] = jnp.concatenate(ts[m], axis=0)
                if not last:
                    @pl.when((i + 1) % GP == 0)
                    def _():
                        start_kv(v_hbm, vb, semv, (i + 1) // GP)
                        wait_group(kb, semk, (i + 1) // GP)

            def step(i, last):
                pl.when(first)(lambda: fetch(i, last))
                e, l = softmax(s_s[...])
                p_s[...] = e
                o_prev = o_red()
                never = jnp.concatenate([z_s[...]] * (GRW // 8), axis=0) != 0
                toks = []
                def add(v, per):
                    for n in range(v.shape[1] // LANES):
                        toks.append(((toks[-1][0] if toks else 0) + per, v[:, n * LANES:(n + 1) * LANES]))
                    return v
                for op in ORDER:
                    if op == 'k' and not last:
                        s_s[...] = add(k_scores(q_s[...], i + 1), 96)
                    elif op == 'q' and not last:
                        q_s[...] = q_lhs(add(q_proj(jnp.minimum(i + 2, NP - 1)), 40))
                    elif op == 'o':
                        acc_s[...] += add(o_proj(o_prev, jnp.maximum(i - 1, 0)), 24)
                    elif op == 'm':
                        o_s[0] = jnp.where(omask, add(pv_mxu(i, e), 8 * NM), 0.0)
                        o_s[1] = jnp.where(omask, jnp.concatenate([l * 0.25] * 3, axis=1), 0.0)
                ng = PAIR // GRW
                for g in range(ng):
                    tm = T0 * 20 + g * (toks[-1][0] - (T0 + T1) * 20) / ng
                    ok = [v for (t_, v) in toks if t_ <= tm]
                    a_s[g * GRW:(g + 1) * GRW, :] = pv_vpu(i, g, never, ok[-1] if ok and not last else None)

            lax.fori_loop(0, NP - 1, lambda i, c_: (step(i, False), c_)[1], 0)
            step(NP - 1, True)
            x1 = _rb(x_s[...] + _rb(acc_s[...] + o_proj(o_red(), NP - 1)))
            @pl.when(first)
            def _():
                wait_all(w1b, sem1.at[0])
            h = _dot(_ln(x1), _cat(w132, NF, 0, D))
            h = _rb(_rb(h) + b1b[...].astype(f32).reshape(1, F))
            h = jax.nn.gelu(h, approximate=True)
            @pl.when(first)
            def _():
                wait_all(w2b, sem2.at[0])
            y = _dot(h, _cat(w232, ND, 0, F))
            y = _rb(_rb(y) + b2b[...].astype(f32).reshape(1, D))
            x_s[...] = _rb(x1 + y)
            return carry
        lax.fori_loop(0, NL, layer, 0)
        o_ref[0] = x_s[0:1, :].astype(o_ref.dtype)

    any_ = pl.BlockSpec(memory_space=pl.ANY)
    return pl.pallas_call(
        kern,
        out_shape=jax.ShapeDtypeStruct((1, 1, D), bf),
        in_specs=[any_] * 9,
        scratch_shapes=[
            pltpu.VMEM((NS, H * DH, LANES), bf), pltpu.VMEM((NS, H * DH + PV, LANES), bf),
            pltpu.VMEM((3 * NP, D, LANES), bf), pltpu.VMEM((ND, H * DH, LANES), bf),
            pltpu.VMEM((NF, D, LANES), bf), pltpu.VMEM((ND, F, LANES), bf),
            pltpu.VMEM((1, 1, D), bf), pltpu.VMEM((F,), bf), pltpu.VMEM((D,), bf),
            pltpu.VMEM((8, D), f32), pltpu.VMEM((8, 4 * PAIR), f32), pltpu.VMEM((8, W // 4), f32),
            pltpu.VMEM((8, W // 4), f32), pltpu.VMEM((PAIR, LANES), f32), pltpu.VMEM((8, LANES), jnp.int32),
            pltpu.VMEM((2, 8, PAIR), f32), pltpu.VMEM((8, D), f32), pltpu.VMEM((8, D), f32),
            pltpu.SemaphoreType.DMA((NG,)), pltpu.SemaphoreType.DMA((NG,)), pltpu.SemaphoreType.DMA((1,)),
            pltpu.SemaphoreType.DMA((1,)), pltpu.SemaphoreType.DMA((1,)), pltpu.SemaphoreType.DMA((1,)),
            pltpu.SemaphoreType.DMA((3,)),
        ],
        compiler_params=pltpu.CompilerParams(vmem_limit_bytes=124 * 1024 * 1024, flags=flags),
        name="fused_layers",
    )


def kernel(A_x, A_k_cache, A_v_cache, A_wq, A_wo, B_x, B_w1, B_b1, B_w2, B_b2, **kw):
    SK = A_k_cache.shape[2]
    W = min(4096, max(256, SK // 4))
    D, F = B_w1.shape
    kt = jnp.swapaxes(A_k_cache, 2, 3).reshape(H * DH, SK)
    vt = jnp.swapaxes(A_v_cache, 2, 3).reshape(H * DH, SK)
    return make(SK, W, D, F, **kw)(A_x, kt, vt, A_wq, A_wo, B_w1, B_b1, B_w2, B_b2)


@jax.jit
def pallas_interleave_layers__sliding_block_cached__dense_activation_gelu__decode_kernel(
    A_x, A_k_cache, A_v_cache, A_wq, A_wo, B_x, B_w1, B_b1, B_w2, B_b2
):
    return kernel(A_x, A_k_cache, A_v_cache, A_wq, A_wo, B_x, B_w1, B_b1, B_w2, B_b2)
```

```python
import jax
import jax.numpy as jnp
from jax import lax
import jax.experimental.pallas as pl
import jax.experimental.pallas.tpu as pltpu

H, DH = 32, 192
PAIR = 2 * DH
NP = H // 2
LANES = 128
bf = jnp.bfloat16
f32 = jnp.float32
u32 = jnp.uint32


def _rb(v):
    return v.astype(bf).astype(f32)


def _ln(x):
    m = jnp.mean(x, axis=-1, keepdims=True)
    d = x - m
    v = jnp.mean(d * d, axis=-1, keepdims=True)
    return d / jnp.sqrt(v + 1e-5)


def _rows32(r0, n):
    h = r0 // 2
    return pl.ds(h if isinstance(h, int) else pl.multiple_of(h, 8), n // 2)


def _tile(ref32, j, r0, n):
    return pltpu.bitcast(ref32[j, _rows32(r0, n), :], bf)


def _cat(ref32, nt, r0, n, base=0):
    return jnp.concatenate([_tile(ref32, base + j, r0, n) for j in range(nt)], axis=1)


def _dot(a, b):
    return lax.dot_general(a, b, (((1,), (0,)), ((), ())), preferred_element_type=f32)


def make(SK, W, D, F, GP=2, NL=2, dma=True, flags=None, NM=10, GRW=32, ORDER='kmqo', T0=4, T1=2, PV=48, U=3, NML=18, PK=16, KO=1):
    NS = W // LANES
    NC = NS // 4
    ND = D // LANES
    NF = F // LANES
    NB = (NP - 1) // U
    korder = [(t, n) for n in range(3) for t in range(4)] if KO else [(t, n) for t in range(4) for n in range(3)]
    c_exp = (DH ** -0.5) * 1.4426950408889634

    def kern(x_hbm, k_hbm, v_hbm, wq_hbm, wo_hbm, w1_hbm, b1_hbm, w2_hbm, b2_hbm, o_ref,
             kb, vb, wqb, wob, w1b, w2b, xb, b1b, b2b, xn_s, q_s, s_s, p_s, a_s, z_s, o_s, acc_s, x_s,
             semk, semv, semq, semo, sem1, sem2, sems):
        kb32, vb32, wq32, w132 = (r.bitcast(u32) for r in (kb, vb, wqb, w1b))

        def start_kv(src, dst, sem, i, n):
            r = pl.ds(i * PAIR if isinstance(i, int) else pl.multiple_of(i * PAIR, PAIR), n * PAIR)
            @pl.loop(0, NS)
            def _(j):
                c = pl.ds(pl.multiple_of(SK - W + j * LANES, LANES), LANES)
                pltpu.make_async_copy(src.at[r, c], dst.at[j, r], sem).start()

        def start_w(src, dst, sem):
            @pl.loop(0, dst.shape[0])
            def _(j):
                c = pl.ds(pl.multiple_of(j * LANES, LANES), LANES)
                pltpu.make_async_copy(src.at[:, c], dst.at[j], sem).start()

        def wait_kv(buf, sem, n):
            t = buf.at[:, pl.ds(0, n * PAIR)]
            pltpu.make_async_copy(t, t, sem).wait()

        def wait_all(buf, sem):
            pltpu.make_async_copy(buf, buf, sem).wait()

        cx = pltpu.make_async_copy(x_hbm, xb, sems.at[0])
        c1 = pltpu.make_async_copy(b1_hbm, b1b, sems.at[1])
        c2 = pltpu.make_async_copy(b2_hbm, b2b, sems.at[2])
        if dma:
            pltpu.make_async_copy(wo_hbm, wob, semo.at[0]).start()
        cx.start(); c1.start(); c2.start()
        if dma:
            start_w(wq_hbm, wqb, semq.at[0])
            start_kv(k_hbm, kb, semk.at[NB], 0, 1)
            start_kv(v_hbm, vb, semv.at[0], 0, U)
            start_kv(k_hbm, kb, semk.at[0], 1, U)
        z_s[...] = jnp.zeros((8, LANES), jnp.int32)
        cx.wait(); c1.wait(); c2.wait()
        x_s[...] = jnp.broadcast_to(xb[0].astype(f32), (8, D))
        if dma:
            wait_all(wob, semo.at[0])
            wait_all(wqb, semq.at[0])
            wait_kv(kb, semk.at[NB], 1)

        row = lax.broadcasted_iota(jnp.int32, (8, 4 * PAIR), 0)
        col = lax.broadcasted_iota(jnp.int32, (8, 4 * PAIR), 1)
        qmask = jnp.logical_and(col >= row * DH, col < (row + 1) * DH)
        row1 = lax.broadcasted_iota(jnp.int32, (8, LANES), 0)
        omask = (lax.broadcasted_iota(jnp.int32, (8, PAIR), 0) & 1) == (
            lax.broadcasted_iota(jnp.int32, (8, PAIR), 1) >= DH).astype(jnp.int32)

        def q_proj(i):
            return _dot(xn_s[...], _cat(wq32, 3, 0, D, base=3 * i))

        def q_lhs(q):
            ql = jnp.where(qmask, jnp.concatenate([_rb(q)] * 4, axis=1), 0.0)
            return jnp.concatenate([ql[:, (3 * t + n) * LANES:(3 * t + n + 1) * LANES] for t, n in korder], axis=1)

        def k_scores(lhs, i):
            rhs = jnp.concatenate(
                [jnp.concatenate([_tile(kb32, 4 * c + t, i * PAIR + n * LANES, LANES) for t, n in korder], axis=0)
                 for c in range(NC)], axis=1)
            return _dot(lhs, rhs)

        def softmax(s):
            m = jnp.max(s, axis=1, keepdims=True)
            m = jnp.broadcast_to(m, (8, LANES))
            m = jnp.maximum(m, pltpu.roll(m, 2, 0))
            m = jnp.maximum(m, pltpu.roll(m, 4, 0))
            e = jnp.exp2((s - jnp.concatenate([m] * NC, axis=1)) * c_exp)
            l = jnp.sum(e, axis=1, keepdims=True)
            l = jnp.broadcast_to(l, (8, LANES))
            l = l + pltpu.roll(l, 2, 0)
            l = l + pltpu.roll(l, 4, 0)
            return e, l

        def pv_vpu(i, u, g, never, tok, nm):
            a = g * GRW // DH
            acc = None
            for j in range(nm, NS):
                c, t = divmod(j, 4)
                p = jnp.broadcast_to(p_s[u, 2 * t + a:2 * t + a + 1, c * LANES:(c + 1) * LANES], (GRW, LANES))
                y = _tile(vb32, j, i * PAIR + g * GRW, GRW).astype(f32) * p
                if acc is None and tok is not None:
                    y = jnp.where(never, jnp.concatenate([tok] * (GRW // 8), axis=0), y)
                acc = y if acc is None else acc + y
            return acc

        def pv_mxu(i, e, nm):
            lhs = jnp.concatenate([jnp.where((row1 >> 1) == j % 4, e[:, (j // 4) * LANES:(j // 4 + 1) * LANES], 0.0)
                                   for j in range(nm)], axis=1)
            rhs = jnp.concatenate(
                [jnp.concatenate([_tile(vb32, j, i * PAIR + n * LANES, LANES) for j in range(nm)], axis=0)
                 for n in range(3)], axis=1)
            return _dot(lhs, rhs)

        def o_red(a, om, ol):
            o = jnp.sum(jnp.concatenate([a.T, om], axis=0), axis=0, keepdims=True)
            l = jnp.sum(ol, axis=0, keepdims=True)
            return jnp.broadcast_to(o / l, (8, PAIR))

        def o_proj(o, i):
            return _dot(o, wob[pl.ds(i * PAIR if isinstance(i, int) else pl.multiple_of(i * PAIR, PAIR), PAIR), :])

        def layer(li, carry):
            first = jnp.logical_and(li == 0, dma)
            xn_s[...] = _ln(x_s[...])
            s_s[...] = k_scores(q_lhs(q_proj(0)), 0)
            q_s[...] = q_lhs(q_proj(1))
            o_s[0] = jnp.zeros((8, PAIR), f32)
            o_s[1] = jnp.ones((8, PAIR), f32)
            a_s[...] = jnp.zeros((PAIR, LANES), f32)
            acc_s[...] = jnp.zeros((8, D), f32)

            def fetch(b):
                wait_kv(vb, semv.at[b], U)
                @pl.when(b + 1 < NB)
                def _():
                    start_kv(v_hbm, vb, semv.at[b + 1], (b + 1) * U, U)
                @pl.when(b + 2 == NB)
                def _():
                    start_kv(v_hbm, vb, semv.at[NB], NP - 1, 1)
                @pl.when(b + 1 == NB)
                def _():
                    start_w(w1_hbm, w1b, sem1.at[0])
                    pltpu.make_async_copy(w2_hbm, w2b, sem2.at[0]).start()
                    wait_kv(vb, semv.at[NB], 1)
                def transpose(i, j):
                    ts = [[pltpu.bitcast(_tile(vb32, j * 2 + m, i * PAIR + n * LANES, LANES).T, u32) for n in range(3)] for m in range(2)]
                    for m in range(2):
                        vb32[j * 2 + m, _rows32(i * PAIR, PAIR), :] = jnp.concatenate(ts[m], axis=0)
                @pl.loop(b * U, jnp.where(b + 1 == NB, NP, (b + 1) * U))
                def _(i):
                    pl.loop(0, jnp.where(i == NP - 1, NML // 2, NM // 2))(lambda j: transpose(i, j))
                wait_kv(kb, semk.at[b], U)
                @pl.when(b + 1 < NB)
                def _():
                    start_kv(k_hbm, kb, semk.at[b + 1], (b + 1) * U + 1, U)

            def steps(i0, n, last):
                nm = NML if last else NM
                never = jnp.concatenate([z_s[...]] * (GRW // 8), axis=0) != 0
                toks = []
                def add(v, per):
                    for m in range(v.shape[1] // LANES):
                        toks.append(((toks[-1][0] if toks else 0) + per, v[:, m * LANES:(m + 1) * LANES]))
                    return v
                s, ql, a, om, ol, acc = s_s[...], q_s[...], a_s[...], o_s[0], o_s[1], acc_s[...]
                ng = PAIR // GRW
                per_step = 8 * (NS * 3 + 6 * ND + 3 * NM)
                t_lo, t_hi = T0 * 20, n * per_step - T1 * 20
                for u in range(n):
                    i = i0 + u
                    e, l = softmax(s)
                    p_s[u] = e
                    o_prev = o_red(a, om, ol)
                    for op in ORDER:
                        if op == 'k' and not last:
                            s = add(k_scores(ql, i + 1), 96)
                        elif op == 'q' and not last:
                            qn = q_lhs(add(q_proj(jnp.minimum(i + 2, NP - 1)), 40))
                        elif op == 'o':
                            acc = acc + add(o_proj(o_prev, jnp.maximum(i - 1, 0)), 24)
                        elif op == 'm':
                            om = jnp.where(omask, add(pv_mxu(i, e, nm), 8 * nm), 0.0)
                            ol = jnp.where(omask, jnp.concatenate([l * 0.25] * 3, axis=1), 0.0)
                    parts = []
                    for g in range(ng):
                        tm = t_lo + (u * ng + g) * (t_hi - t_lo) / (n * ng)
                        ok = [v for (t_, v) in toks if t_ <= tm]
                        parts.append(pv_vpu(i, u, g, never, ok[-1] if ok and not last else None, nm))
                    a = jnp.concatenate(parts, axis=0)
                    if not last:
                        ql = qn
                if last:
                    return acc + o_proj(o_red(a, om, ol), NP - 1)
                s_s[...], q_s[...], a_s[...], o_s[0], o_s[1], acc_s[...] = s, ql, a, om, ol, acc

            @pl.loop(0, NB)
            def _(b):
                pl.when(first)(lambda: fetch(b))
                steps(b * U, U, False)
            attn = steps(NP - 1, 1, True)
            x1 = _rb(x_s[...] + _rb(attn))
            @pl.when(first)
            def _():
                wait_all(w1b, sem1.at[0])
            h = _dot(_ln(x1), _cat(w132, NF, 0, D))
            h = _rb(_rb(h) + b1b[...].astype(f32).reshape(1, F))
            h = jax.nn.gelu(h, approximate=True)
            @pl.when(first)
            def _():
                wait_all(w2b, sem2.at[0])
            y = _dot(h, w2b[...])
            y = _rb(_rb(y) + b2b[...].astype(f32).reshape(1, D))
            x_s[...] = _rb(x1 + y)
            return carry
        lax.fori_loop(0, NL, layer, 0)
        o_ref[0] = x_s[0:1, :].astype(o_ref.dtype)

    any_ = pl.BlockSpec(memory_space=pl.ANY)
    return pl.pallas_call(
        kern,
        out_shape=jax.ShapeDtypeStruct((1, 1, D), bf),
        in_specs=[any_] * 9,
        scratch_shapes=[
            pltpu.VMEM((NS, H * DH + PK, LANES), bf), pltpu.VMEM((NS, H * DH + PV, LANES), bf),
            pltpu.VMEM((3 * NP, D, LANES), bf), pltpu.VMEM((H * DH, D), bf),
            pltpu.VMEM((NF, D, LANES), bf), pltpu.VMEM((F, D), bf),
            pltpu.VMEM((1, 1, D), bf), pltpu.VMEM((F,), bf), pltpu.VMEM((D,), bf),
            pltpu.VMEM((8, D), f32), pltpu.VMEM((8, 4 * PAIR), f32), pltpu.VMEM((8, W // 4), f32),
            pltpu.VMEM((U, 8, W // 4), f32), pltpu.VMEM((PAIR, LANES), f32), pltpu.VMEM((8, LANES), jnp.int32),
            pltpu.VMEM((2, 8, PAIR), f32), pltpu.VMEM((8, D), f32), pltpu.VMEM((8, D), f32),
            pltpu.SemaphoreType.DMA((NB + 1,)), pltpu.SemaphoreType.DMA((NB + 1,)), pltpu.SemaphoreType.DMA((1,)),
            pltpu.SemaphoreType.DMA((1,)), pltpu.SemaphoreType.DMA((1,)), pltpu.SemaphoreType.DMA((1,)),
            pltpu.SemaphoreType.DMA((3,)),
        ],
        compiler_params=pltpu.CompilerParams(vmem_limit_bytes=124 * 1024 * 1024, flags=flags),
        name="fused_layers",
    )


def kernel(A_x, A_k_cache, A_v_cache, A_wq, A_wo, B_x, B_w1, B_b1, B_w2, B_b2, **kw):
    SK = A_k_cache.shape[2]
    W = min(4096, max(256, SK // 4))
    D, F = B_w1.shape
    kt = jnp.swapaxes(A_k_cache, 2, 3).reshape(H * DH, SK)
    vt = jnp.swapaxes(A_v_cache, 2, 3).reshape(H * DH, SK)
    return make(SK, W, D, F, **kw)(A_x, kt, vt, A_wq, A_wo, B_w1, B_b1, B_w2, B_b2)


@jax.jit
def pallas_interleave_layers__sliding_block_cached__dense_activation_gelu__decode_kernel(
    A_x, A_k_cache, A_v_cache, A_wq, A_wo, B_x, B_w1, B_b1, B_w2, B_b2
):
    return kernel(A_x, A_k_cache, A_v_cache, A_wq, A_wo, B_x, B_w1, B_b1, B_w2, B_b2)
```

```python
import jax
import jax.numpy as jnp
from jax import lax
import jax.experimental.pallas as pl
import jax.experimental.pallas.tpu as pltpu

H, DH = 32, 192
PAIR = 2 * DH
NP = H // 2
LANES = 128
NSLAB = H * DH // LANES
U = 3
NB = (NP - 1) // U
VROWS = 32
bf16, f32, u32 = jnp.bfloat16, jnp.float32, jnp.uint32


def _round(v):
    return v.astype(bf16).astype(f32)


def _layernorm(x):
    d = x - jnp.mean(x, axis=-1, keepdims=True)
    return d / jnp.sqrt(jnp.mean(d * d, axis=-1, keepdims=True) + 1e-5)


def _ds(start, size, align):
    return pl.ds(start if isinstance(start, int) else pl.multiple_of(start, align), size)


def _tile(ref32, j, r0, n):
    return pltpu.bitcast(ref32[j, _ds(r0 // 2, n // 2, 8), :], bf16)


def _tiles(ref32, j0, nj, r0, n):
    return jnp.concatenate([_tile(ref32, j0 + j, r0, n) for j in range(nj)], axis=1)


def _lane_tile(v, m):
    return v[:, m * LANES:(m + 1) * LANES]


def _dot(a, b):
    return lax.dot_general(a, b, (((1,), (0,)), ((), ())), preferred_element_type=f32)


class _Copy:
    def __init__(self, src, dst, sem, pieces):
        self.src, self.dst, self.sem, self.pieces = src, dst, sem, pieces

    def start(self):
        n = self.dst.shape[0] // self.pieces

        @pl.loop(0, self.pieces)
        def _(p):
            rows = _ds(p * n, n, n)
            pltpu.make_async_copy(self.src.at[rows], self.dst.at[rows], self.sem).start()

    def wait(self):
        pltpu.make_async_copy(self.src, self.dst, self.sem).wait()


def _iota(shape, axis):
    return lax.broadcasted_iota(jnp.int32, shape, axis)


def _build(SK, W, D, F, NM=6, NML=18, NT=3, T0=0, T1=20, NL=2, RING=3, SPL=4, SPW=8, interpret=False):
    NS, ND, NF = W // LANES, D // LANES, F // LANES
    NC, NQ = NS // 4, H * DH // F
    assert F == (U + 1) * PAIR and NS % 4 == 0 and NM % 2 == 0 and NML % NM == 0 and NML < NS
    exp_scale = (DH ** -0.5) * 1.4426950408889634

    def body(x_hbm, k_hbm, v_hbm, wq_hbm, wo_hbm, w1_hbm, b1_hbm, w2_hbm, b2_hbm, out_ref,
             kb32, vb32, wq32, wo32, kring, vring, w1b, w2b, xb, b1b, b2b,
             x_s, xn_s, q_s, s_s, p_s, a_s, o_s, acc_s, zero_s,
             semk, semv, semw):
        def slab_copies(m):
            rows, slot = _ds(m * LANES, LANES, LANES), m % RING
            return [_Copy(src.at[rows, pl.ds(SK - W, W)], ring.at[slot], sem.at[slot], SPL)
                    for src, ring, sem in ((v_hbm, vring, semv), (k_hbm, kring, semk))]

        def wq_copy(c):
            return _Copy(wq_hbm.at[:, _ds(c * F, F, LANES)], w1b, semw.at[0], SPW)

        def wo_copy(i, n, staged):
            return _Copy(
                wo_hbm.at[_ds(i * PAIR, n * PAIR, PAIR)], w2b.at[pl.ds(staged * PAIR, n * PAIR)],
                semw.at[1 + staged // U], SPW)

        w1_copy = _Copy(w1_hbm, w1b, semw.at[0], SPW)
        w2_copy = _Copy(w2_hbm, w2b, semw.at[1], SPW)
        small = [pltpu.make_async_copy(s, d, semw.at[3 + n])
                 for n, (s, d) in enumerate(((x_hbm, xb), (b1_hbm, b1b), (b2_hbm, b2b)))]

        def pack_wq(c):
            wq_copy(c).wait()

            @pl.loop(0, NF)
            def _(j):
                wq32[c * NF + j] = pltpu.bitcast(w1b[:, _ds(j * LANES, LANES, LANES)], u32)

        def pack_wo(i, staged):
            @pl.loop(0, ND)
            def _(j):
                w = w2b[_ds(staged * PAIR, PAIR, PAIR), _ds(j * LANES, LANES, LANES)]
                wo32[j, _ds(i * DH, DH, 8), :] = pltpu.bitcast(w, u32)

        def pack_slab(m):
            def pack(dst, ring, lo, hi, step, transpose=False):
                @pl.loop(lo, hi)
                def _(g):
                    for j in range(step):
                        t = ring[m % RING, :, _ds((g * step + j) * LANES, LANES, LANES)]
                        dst[g * step + j, _ds(m * (LANES // 2), LANES // 2, 8), :] = pltpu.bitcast(
                            t.T if transpose else t, u32)

            v_copy, k_copy = slab_copies(m)
            last = m >= NSLAB - 3
            v_copy.wait()
            pack(vb32, vring, 0, jnp.where(last, NML // NM, 1), NM, True)
            pack(vb32, vring, jnp.where(last, NML // 2, NM // 2), NS // 2, 2)
            k_copy.wait()
            pack(kb32, kring, 0, NC, 4)

            @pl.when(m + RING < NSLAB)
            def _():
                for c in slab_copies(m + RING):
                    c.start()

            @pl.when(m + RING == NSLAB - 1)
            def _():
                w1_copy.start()
                w2_copy.start()

        def fetch(b):
            wo_copy(b * U, U, 0).wait()
            pl.loop(0, U)(lambda u: pack_wo(b * U + u, u))
            pl.when(b + 1 < NB)(lambda: wo_copy((b + 1) * U, U, 0).start())

            @pl.when(b + 1 < NQ)
            def _():
                pack_wq(b + 1)
                pl.when(b + 2 < NQ)(lambda: wq_copy(b + 2).start())

            pl.loop(3 * (b * U + 1), 3 * (b * U + 1 + U))(pack_slab)

        for m in range(RING):
            for c in slab_copies(m):
                c.start()
        for c in small + [wq_copy(0), wo_copy(0, U, 0), wo_copy(NP - 1, 1, U)]:
            c.start()
        zero_s[...] = jnp.zeros((8, LANES), jnp.int32)
        pl.loop(0, 3)(pack_slab)
        for c in small:
            c.wait()
        x_s[...] = jnp.broadcast_to(xb[0].astype(f32), (8, D))
        pack_wq(0)
        wq_copy(1).start()
        wo_copy(NP - 1, 1, U).wait()
        pack_wo(NP - 1, U)

        row = _iota((8, LANES), 0)
        upper = (_iota((8, LANES), 1) >= DH - LANES).astype(jnp.int32)
        head_of_lane = [(n + upper) >> 1 for n in range(3)]
        own_head = jnp.concatenate([(row & 1) - h for h in head_of_lane], axis=1) == 0

        def q_proj(i):
            return _dot(xn_s[...], _tiles(wq32, 3 * i, 3, 0, D))

        def q_blocks(q):
            q = _round(q)
            return jnp.concatenate(
                [jnp.where(row == 2 * t + head_of_lane[n], _lane_tile(q, n), 0.0)
                 for n in range(3) for t in range(4)], axis=1)

        def scores(q, i, mark=lambda v, cost: v):
            cols = []
            for c in range(NC):
                y = None
                for n in range(3):
                    k = jnp.concatenate(
                        [_tile(kb32, 4 * c + t, i * PAIR + n * LANES, LANES) for t in range(4)], axis=0)
                    z = _dot(q[:, 4 * n * LANES:4 * (n + 1) * LANES], k)
                    y = mark(z if y is None else y + z, 4)
                cols.append(y)
            return jnp.concatenate(cols, axis=1)

        def per_head(v, op):
            v = jnp.broadcast_to(v, (8, LANES))
            v = op(v, pltpu.roll(v, 2, 0))
            return op(v, pltpu.roll(v, 4, 0))

        def softmax(s):
            m = per_head(jnp.max(s, axis=1, keepdims=True), jnp.maximum)
            e = jnp.exp2((s - jnp.concatenate([m] * NC, axis=1)) * exp_scale)
            return e, per_head(jnp.sum(e, axis=1, keepdims=True), jnp.add)

        def pv_mxu(i, e, nm):
            p = jnp.concatenate(
                [jnp.where((row >> 1) == j % 4, _lane_tile(e, j // 4), 0.0) for j in range(nm)], axis=1)
            v = jnp.concatenate(
                [jnp.concatenate([_tile(vb32, j, i * PAIR + n * LANES, LANES) for j in range(nm)], axis=0)
                 for n in range(3)], axis=1)
            return _dot(p, v)

        def pv_vpu(i, u, g, nm, never, after):
            a = g * VROWS // DH
            acc = None
            for j in range(nm, NS):
                c, t = divmod(j, 4)
                p = p_s[u, 2 * t + a:2 * t + a + 1, c * LANES:(c + 1) * LANES]
                y = _tile(vb32, j, i * PAIR + g * VROWS, VROWS).astype(f32) * jnp.broadcast_to(p, (VROWS, LANES))
                seg, off = divmod(j - nm, pl.cdiv(NS - nm, NT))
                if off == 0 and after[seg] is not None:
                    y = jnp.where(never, jnp.concatenate([after[seg]] * (VROWS // 8), axis=0), y)
                acc = y if acc is None else acc + y
            return acc

        def head_out(a, om, ol):
            o = jnp.sum(jnp.concatenate([a.T, om], axis=0), axis=0, keepdims=True)
            return jnp.broadcast_to(o / jnp.sum(ol, axis=0, keepdims=True), (8, PAIR))

        def o_proj(o, i):
            return _dot(o, _tiles(wo32, 0, ND, i * PAIR, PAIR))

        def attend(i0, n, last):
            nm = NML if last else NM
            never = jnp.concatenate([zero_s[...]] * (VROWS // 8), axis=0) != 0
            marks = []

            def mark(v, tiles):
                for m in range(v.shape[1] // LANES):
                    marks.append(((marks[-1][0] if marks else 0) + 8 * tiles, _lane_tile(v, m)))
                return v

            s, q, a, om, ol, acc = s_s[...], q_s[...], a_s[...], o_s[0], o_s[1], acc_s[...]
            ng = PAIR // VROWS
            span = n * 8 * (3 * NS + 6 * ND + 3 * nm) - T0 - T1
            for u in range(n):
                i = i0 + u
                e, l = softmax(s)
                p_s[u] = e
                o_prev = head_out(a, om, ol)
                if not last:
                    s = scores(q, i + 1, mark)
                om = jnp.where(own_head, mark(pv_mxu(i, e, nm), nm), 0.0)
                ol = jnp.where(own_head, jnp.concatenate([l * 0.25] * 3, axis=1), 0.0)
                if not last:
                    q = q_blocks(mark(q_proj(jnp.minimum(i + 2, NP - 1)), ND))
                acc = acc + mark(o_proj(o_prev, jnp.maximum(i - 1, 0)), 3)
                parts = []
                for g in range(ng):
                    ready = [0] + [sum(t <= T0 + (u * ng + g + seg / NT) * span / (n * ng) for t, _ in marks)
                                   for seg in range(NT)]
                    after = [marks[r - 1][1] if r > r0 and not last else None
                             for r0, r in zip(ready, ready[1:])]
                    parts.append(pv_vpu(i, u, g, nm, never, after))
                a = jnp.concatenate(parts, axis=0)
            if last:
                return acc + o_proj(head_out(a, om, ol), i0)
            s_s[...], q_s[...], a_s[...], o_s[0], o_s[1], acc_s[...] = s, q, a, om, ol, acc

        @pl.loop(0, NL)
        def _(layer):
            first = layer == 0
            xn_s[...] = _layernorm(x_s[...])
            s_s[...] = scores(q_blocks(q_proj(0)), 0)
            q_s[...] = q_blocks(q_proj(1))
            a_s[...] = jnp.zeros((PAIR, LANES), f32)
            o_s[0] = jnp.zeros((8, PAIR), f32)
            o_s[1] = jnp.ones((8, PAIR), f32)
            acc_s[...] = jnp.zeros((8, D), f32)

            @pl.loop(0, NB)
            def _(b):
                pl.when(first)(lambda: fetch(b))
                attend(b * U, U, False)

            x = _round(x_s[...] + _round(attend(NP - 1, 1, True)))
            pl.when(first)(w1_copy.wait)
            h = _dot(_layernorm(x), w1b[...])
            h = _round(_round(h) + b1b[...].astype(f32).reshape(1, F))
            h = jax.nn.gelu(h, approximate=True)
            pl.when(first)(w2_copy.wait)
            y = _round(_round(_dot(h, w2b[...])) + b2b[...].astype(f32).reshape(1, D))
            x_s[...] = _round(x + y)

        out_ref[0] = x_s[0:1, :].astype(out_ref.dtype)

    vmem, dma = pltpu.VMEM, pltpu.SemaphoreType.DMA
    return pl.pallas_call(
        body,
        out_shape=jax.ShapeDtypeStruct((1, 1, D), bf16),
        in_specs=[pl.BlockSpec(memory_space=pl.ANY)] * 9,
        scratch_shapes=[
            vmem((NS, H * DH // 2 + 8, LANES), u32), vmem((NS, H * DH // 2 + 24, LANES), u32),
            vmem((NSLAB, D // 2, LANES), u32), vmem((ND, H * DH // 2, LANES), u32),
            vmem((RING, LANES, W), bf16), vmem((RING, LANES, W), bf16),
            vmem((D, F), bf16), vmem((F, D), bf16),
            vmem((1, 1, D), bf16), vmem((F,), bf16), vmem((D,), bf16),
            vmem((8, D), f32), vmem((8, D), f32), vmem((8, 4 * PAIR), f32), vmem((8, W // 4), f32),
            vmem((U, 8, W // 4), f32), vmem((PAIR, LANES), f32), vmem((2, 8, PAIR), f32),
            vmem((8, D), f32), vmem((8, LANES), jnp.int32),
            dma((RING,)), dma((RING,)), dma((6,)),
        ],
        compiler_params=pltpu.CompilerParams(vmem_limit_bytes=124 * 1024 * 1024),
        interpret=interpret,
        name="fused_layers",
    )


def kernel(A_x, A_k_cache, A_v_cache, A_wq, A_wo, B_x, B_w1, B_b1, B_w2, B_b2, **kw):
    del B_x
    SK = A_k_cache.shape[2]
    W = min(4096, max(256, SK // 4))
    D, F = B_w1.shape
    kt = jnp.swapaxes(A_k_cache, 2, 3).reshape(H * DH, SK)
    vt = jnp.swapaxes(A_v_cache, 2, 3).reshape(H * DH, SK)
    return _build(SK, W, D, F, **kw)(A_x, kt, vt, A_wq, A_wo, B_w1, B_b1, B_w2, B_b2)


@jax.jit
def pallas_interleave_layers__sliding_block_cached__dense_activation_gelu__decode_kernel(
    A_x, A_k_cache, A_v_cache, A_wq, A_wo, B_x, B_w1, B_b1, B_w2, B_b2
):
    return kernel(A_x, A_k_cache, A_v_cache, A_wq, A_wo, B_x, B_w1, B_b1, B_w2, B_b2)
```

```python
import jax
import jax.numpy as jnp
from jax import lax
import jax.experimental.pallas as pl
import jax.experimental.pallas.tpu as pltpu

H, DH = 32, 192
PAIR = 2 * DH
NP = H // 2
LANES = 128
NSLAB = H * DH // LANES
U = 3
NB = (NP - 1) // U
VROWS = 32
NT = 3
RING = 3
SPL, SPW = 4, 8
bf16, f32, u32 = jnp.bfloat16, jnp.float32, jnp.uint32


def _round(v):
    return v.astype(bf16).astype(f32)


def _layernorm(x):
    d = x - jnp.mean(x, axis=-1, keepdims=True)
    return d / jnp.sqrt(jnp.mean(d * d, axis=-1, keepdims=True) + 1e-5)


def _ds(start, size, align):
    return pl.ds(start if isinstance(start, int) else pl.multiple_of(start, align), size)


def _tile(ref32, j, r0, n):
    return pltpu.bitcast(ref32[j, _ds(r0 // 2, n // 2, 8), :], bf16)


def _tiles(ref32, j0, nj, r0, n):
    return jnp.concatenate([_tile(ref32, j0 + j, r0, n) for j in range(nj)], axis=1)


def _lane_tile(v, m):
    return v[:, m * LANES:(m + 1) * LANES]


def _dot(a, b):
    return lax.dot_general(a, b, (((1,), (0,)), ((), ())), preferred_element_type=f32)


class _Copy:
    def __init__(self, src, dst, sem, pieces):
        self.src, self.dst, self.sem, self.pieces = src, dst, sem, pieces

    def start(self):
        n = self.dst.shape[0] // self.pieces

        @pl.loop(0, self.pieces)
        def _(p):
            rows = _ds(p * n, n, n)
            pltpu.make_async_copy(self.src.at[rows], self.dst.at[rows], self.sem).start()

    def wait(self):
        pltpu.make_async_copy(self.src, self.dst, self.sem).wait()


def _iota(shape, axis):
    return lax.broadcasted_iota(jnp.int32, shape, axis)


def _build(SK, W, D, F):
    NS, ND, NF = W // LANES, D // LANES, F // LANES
    NC, NQ = NS // 4, H * DH // F
    NM, NML = (6, 18) if NS == 32 else (2, 2)
    assert F == (U + 1) * PAIR and NS % 4 == 0 and NM % 2 == 0 and NML % NM == 0 and NML < NS
    exp_scale = (DH ** -0.5) * 1.4426950408889634

    def body(x_hbm, k_hbm, v_hbm, wq_hbm, wo_hbm, w1_hbm, b1_hbm, w2_hbm, b2_hbm, out_ref,
             kb32, vb32, wq32, wo32, kring, vring, w1b, w2b, xb, b1b, b2b,
             x_s, xn_s, q_s, s_s, p_s, a_s, o_s, acc_s, zero_s,
             semk, semv, semw):
        def slab_copies(m):
            rows, slot = _ds(m * LANES, LANES, LANES), m % RING
            return [_Copy(src.at[rows, pl.ds(SK - W, W)], ring.at[slot], sem.at[slot], SPL)
                    for src, ring, sem in ((v_hbm, vring, semv), (k_hbm, kring, semk))]

        def wq_copy(c):
            return _Copy(wq_hbm.at[:, _ds(c * F, F, LANES)], w1b, semw.at[0], SPW)

        def wo_copy(i, n, staged):
            return _Copy(
                wo_hbm.at[_ds(i * PAIR, n * PAIR, PAIR)], w2b.at[pl.ds(staged * PAIR, n * PAIR)],
                semw.at[1 + staged // U], SPW)

        w1_copy = _Copy(w1_hbm, w1b, semw.at[0], SPW)
        w2_copy = _Copy(w2_hbm, w2b, semw.at[1], SPW)
        small = [pltpu.make_async_copy(s, d, semw.at[3 + n])
                 for n, (s, d) in enumerate(((x_hbm, xb), (b1_hbm, b1b), (b2_hbm, b2b)))]

        def pack_wq(c):
            wq_copy(c).wait()

            @pl.loop(0, NF)
            def _(j):
                wq32[c * NF + j] = pltpu.bitcast(w1b[:, _ds(j * LANES, LANES, LANES)], u32)

        def pack_wo(i, staged):
            @pl.loop(0, ND)
            def _(j):
                w = w2b[_ds(staged * PAIR, PAIR, PAIR), _ds(j * LANES, LANES, LANES)]
                wo32[j, _ds(i * DH, DH, 8), :] = pltpu.bitcast(w, u32)

        def pack_slab(m):
            def pack(dst, ring, lo, hi, step, transpose=False):
                @pl.loop(lo, hi)
                def _(g):
                    for j in range(step):
                        t = ring[m % RING, :, _ds((g * step + j) * LANES, LANES, LANES)]
                        dst[g * step + j, _ds(m * (LANES // 2), LANES // 2, 8), :] = pltpu.bitcast(
                            t.T if transpose else t, u32)

            v_copy, k_copy = slab_copies(m)
            last = m >= NSLAB - 3
            v_copy.wait()
            pack(vb32, vring, 0, jnp.where(last, NML // NM, 1), NM, True)
            pack(vb32, vring, jnp.where(last, NML // 2, NM // 2), NS // 2, 2)
            k_copy.wait()
            pack(kb32, kring, 0, NC, 4)

            @pl.when(m + RING < NSLAB)
            def _():
                for c in slab_copies(m + RING):
                    c.start()

            @pl.when(m + RING == NSLAB - 1)
            def _():
                w1_copy.start()
                w2_copy.start()

        def fetch(b):
            wo_copy(b * U, U, 0).wait()
            pl.loop(0, U)(lambda u: pack_wo(b * U + u, u))
            pl.when(b + 1 < NB)(lambda: wo_copy((b + 1) * U, U, 0).start())

            @pl.when(b + 1 < NQ)
            def _():
                pack_wq(b + 1)
                pl.when(b + 2 < NQ)(lambda: wq_copy(b + 2).start())

            pl.loop(3 * (b * U + 1), 3 * (b * U + 1 + U))(pack_slab)

        for m in range(RING):
            for c in slab_copies(m):
                c.start()
        for c in small + [wq_copy(0), wo_copy(0, U, 0), wo_copy(NP - 1, 1, U)]:
            c.start()
        zero_s[...] = jnp.zeros((8, LANES), jnp.int32)
        pl.loop(0, 3)(pack_slab)
        for c in small:
            c.wait()
        x_s[...] = jnp.broadcast_to(xb[0].astype(f32), (8, D))
        pack_wq(0)
        wq_copy(1).start()
        wo_copy(NP - 1, 1, U).wait()
        pack_wo(NP - 1, U)

        row = _iota((8, LANES), 0)
        upper = (_iota((8, LANES), 1) >= DH - LANES).astype(jnp.int32)
        head_of_lane = [(n + upper) >> 1 for n in range(3)]
        own_head = jnp.concatenate([(row & 1) - h for h in head_of_lane], axis=1) == 0

        def q_proj(i):
            return _dot(xn_s[...], _tiles(wq32, 3 * i, 3, 0, D))

        def q_blocks(q):
            q = _round(q)
            return jnp.concatenate(
                [jnp.where(row == 2 * t + head_of_lane[n], _lane_tile(q, n), 0.0)
                 for n in range(3) for t in range(4)], axis=1)

        def scores(q, i, mark=lambda v, cost: v):
            cols = []
            for c in range(NC):
                y = None
                for n in range(3):
                    k = jnp.concatenate(
                        [_tile(kb32, 4 * c + t, i * PAIR + n * LANES, LANES) for t in range(4)], axis=0)
                    z = _dot(q[:, 4 * n * LANES:4 * (n + 1) * LANES], k)
                    y = mark(z if y is None else y + z, 4)
                cols.append(y)
            return jnp.concatenate(cols, axis=1)

        def per_head(v, op):
            v = jnp.broadcast_to(v, (8, LANES))
            v = op(v, pltpu.roll(v, 2, 0))
            return op(v, pltpu.roll(v, 4, 0))

        def softmax(s):
            m = per_head(jnp.max(s, axis=1, keepdims=True), jnp.maximum)
            e = jnp.exp2((s - jnp.concatenate([m] * NC, axis=1)) * exp_scale)
            return e, per_head(jnp.sum(e, axis=1, keepdims=True), jnp.add)

        def pv_mxu(i, e, nm):
            p = jnp.concatenate(
                [jnp.where((row >> 1) == j % 4, _lane_tile(e, j // 4), 0.0) for j in range(nm)], axis=1)
            v = jnp.concatenate(
                [jnp.concatenate([_tile(vb32, j, i * PAIR + n * LANES, LANES) for j in range(nm)], axis=0)
                 for n in range(3)], axis=1)
            return _dot(p, v)

        def pv_vpu(i, u, g, nm, never, after):
            a = g * VROWS // DH
            acc = None
            for j in range(nm, NS):
                c, t = divmod(j, 4)
                p = p_s[u, 2 * t + a:2 * t + a + 1, c * LANES:(c + 1) * LANES]
                y = _tile(vb32, j, i * PAIR + g * VROWS, VROWS).astype(f32) * jnp.broadcast_to(p, (VROWS, LANES))
                seg, off = divmod(j - nm, pl.cdiv(NS - nm, NT))
                if off == 0 and after[seg] is not None:
                    y = jnp.where(never, jnp.concatenate([after[seg]] * (VROWS // 8), axis=0), y)
                acc = y if acc is None else acc + y
            return acc

        def head_out(a, om, ol):
            o = jnp.sum(jnp.concatenate([a.T, om], axis=0), axis=0, keepdims=True)
            return jnp.broadcast_to(o / jnp.sum(ol, axis=0, keepdims=True), (8, PAIR))

        def o_proj(o, i):
            return _dot(o, _tiles(wo32, 0, ND, i * PAIR, PAIR))

        def attend(i0, n, last):
            nm = NML if last else NM
            never = jnp.concatenate([zero_s[...]] * (VROWS // 8), axis=0) != 0
            marks = []

            def mark(v, tiles):
                for m in range(v.shape[1] // LANES):
                    marks.append(((marks[-1][0] if marks else 0) + 8 * tiles, _lane_tile(v, m)))
                return v

            s, q, a, om, ol, acc = s_s[...], q_s[...], a_s[...], o_s[0], o_s[1], acc_s[...]
            ng = PAIR // VROWS
            span = n * 8 * (3 * NS + 6 * ND + 3 * nm) - 40
            for u in range(n):
                i = i0 + u
                e, l = softmax(s)
                p_s[u] = e
                o_prev = head_out(a, om, ol)
                if not last:
                    s = scores(q, i + 1, mark)
                om = jnp.where(own_head, mark(pv_mxu(i, e, nm), nm), 0.0)
                ol = jnp.where(own_head, jnp.concatenate([l * 0.25] * 3, axis=1), 0.0)
                if not last:
                    q = q_blocks(mark(q_proj(jnp.minimum(i + 2, NP - 1)), ND))
                acc = acc + mark(o_proj(o_prev, jnp.maximum(i - 1, 0)), 3)
                parts = []
                for g in range(ng):
                    ready = [0] + [sum(t <= (u * ng + g + seg / NT) * span / (n * ng) for t, _ in marks)
                                   for seg in range(NT)]
                    after = [marks[r - 1][1] if r > r0 and not last else None
                             for r0, r in zip(ready, ready[1:])]
                    parts.append(pv_vpu(i, u, g, nm, never, after))
                a = jnp.concatenate(parts, axis=0)
            if last:
                return acc + o_proj(head_out(a, om, ol), i0)
            s_s[...], q_s[...], a_s[...], o_s[0], o_s[1], acc_s[...] = s, q, a, om, ol, acc

        @pl.loop(0, 2)
        def _(layer):
            first = layer == 0
            xn_s[...] = _layernorm(x_s[...])
            s_s[...] = scores(q_blocks(q_proj(0)), 0)
            q_s[...] = q_blocks(q_proj(1))
            a_s[...] = jnp.zeros((PAIR, LANES), f32)
            o_s[0] = jnp.zeros((8, PAIR), f32)
            o_s[1] = jnp.ones((8, PAIR), f32)
            acc_s[...] = jnp.zeros((8, D), f32)

            @pl.loop(0, NB)
            def _(b):
                pl.when(first)(lambda: fetch(b))
                attend(b * U, U, False)

            x = _round(x_s[...] + _round(attend(NP - 1, 1, True)))
            pl.when(first)(w1_copy.wait)
            h = _dot(_layernorm(x), w1b[...])
            h = _round(_round(h) + b1b[...].astype(f32).reshape(1, F))
            h = jax.nn.gelu(h, approximate=True)
            pl.when(first)(w2_copy.wait)
            y = _round(_round(_dot(h, w2b[...])) + b2b[...].astype(f32).reshape(1, D))
            x_s[...] = _round(x + y)

        out_ref[0] = x_s[0:1, :].astype(out_ref.dtype)

    vmem, dma = pltpu.VMEM, pltpu.SemaphoreType.DMA
    return pl.pallas_call(
        body,
        out_shape=jax.ShapeDtypeStruct((1, 1, D), bf16),
        in_specs=[pl.BlockSpec(memory_space=pl.ANY)] * 9,
        scratch_shapes=[
            vmem((NS, H * DH // 2 + 8, LANES), u32), vmem((NS, H * DH // 2 + 24, LANES), u32),
            vmem((NSLAB, D // 2, LANES), u32), vmem((ND, H * DH // 2, LANES), u32),
            vmem((RING, LANES, W), bf16), vmem((RING, LANES, W), bf16),
            vmem((D, F), bf16), vmem((F, D), bf16),
            vmem((1, 1, D), bf16), vmem((F,), bf16), vmem((D,), bf16),
            vmem((8, D), f32), vmem((8, D), f32), vmem((8, 4 * PAIR), f32), vmem((8, W // 4), f32),
            vmem((U, 8, W // 4), f32), vmem((PAIR, LANES), f32), vmem((2, 8, PAIR), f32),
            vmem((8, D), f32), vmem((8, LANES), jnp.int32),
            dma((RING,)), dma((RING,)), dma((6,)),
        ],
        compiler_params=pltpu.CompilerParams(vmem_limit_bytes=124 * 1024 * 1024),
        name="fused_layers",
    )


@jax.jit
def pallas_interleave_layers__sliding_block_cached__dense_activation_gelu__decode_kernel(
    A_x: jax.Array,
    A_k_cache: jax.Array,
    A_v_cache: jax.Array,
    A_wq: jax.Array,
    A_wo: jax.Array,
    B_x: jax.Array,
    B_w1: jax.Array,
    B_b1: jax.Array,
    B_w2: jax.Array,
    B_b2: jax.Array,
):
    del B_x
    SK = A_k_cache.shape[2]
    W = min(4096, max(256, SK // 4))
    D, F = B_w1.shape
    kt = jnp.swapaxes(A_k_cache, 2, 3).reshape(H * DH, SK)
    vt = jnp.swapaxes(A_v_cache, 2, 3).reshape(H * DH, SK)
    return _build(SK, W, D, F)(A_x, kt, vt, A_wq, A_wo, B_w1, B_b1, B_w2, B_b2)
```

```python
import jax
import jax.numpy as jnp
from jax import lax
import jax.experimental.pallas as pl
import jax.experimental.pallas.tpu as pltpu

H, DH = 32, 192
PAIR = 2 * DH
NP = H // 2
LANES = 128
NSLAB = H * DH // LANES
U = 3
NB = (NP - 1) // U
VROWS = 32
NT = 3
RING = 2
SPL, SPW = 4, 8
NW = 4
bf16, f32, u32 = jnp.bfloat16, jnp.float32, jnp.uint32


def _round(v):
    return v.astype(bf16).astype(f32)


def _layernorm(x):
    d = x - jnp.mean(x, axis=-1, keepdims=True)
    return d / jnp.sqrt(jnp.mean(d * d, axis=-1, keepdims=True) + 1e-5)


def _ds(start, size, align):
    return pl.ds(start if isinstance(start, int) else pl.multiple_of(start, align), size)


def _tile(ref32, j, r0, n):
    return pltpu.bitcast(ref32[j, _ds(r0 // 2, n // 2, 8), :], bf16)


def _tiles(ref32, j0, nj, r0, n):
    return jnp.concatenate([_tile(ref32, j0 + j, r0, n) for j in range(nj)], axis=1)


def _lane_tile(v, m):
    return v[:, m * LANES:(m + 1) * LANES]


def _dot(a, b):
    return lax.dot_general(a, b, (((1,), (0,)), ((), ())), preferred_element_type=f32)


class _Copy:
    def __init__(self, src, dst, sem, pieces):
        self.src, self.dst, self.sem, self.pieces = src, dst, sem, pieces

    def start(self):
        n = self.dst.shape[0] // self.pieces

        @pl.loop(0, self.pieces)
        def _(p):
            rows = _ds(p * n, n, n)
            pltpu.make_async_copy(self.src.at[rows], self.dst.at[rows], self.sem).start()

    def wait(self):
        pltpu.make_async_copy(self.src, self.dst, self.sem).wait()


def _iota(shape, axis):
    return lax.broadcasted_iota(jnp.int32, shape, axis)


def _build(SK, W, D, F):
    NS, ND, NF = W // LANES, D // LANES, F // LANES
    NC, NQ = NS // 4, H * DH // F
    NM, NML = (6, 18) if NS == 32 else (2, 2)
    assert F == (U + 1) * PAIR and NS % 4 == 0 and NM % 2 == 0 and NML % NM == 0 and NML < NS
    exp_scale = (DH ** -0.5) * 1.4426950408889634

    def body(x_hbm, k_hbm, v_hbm, wq_hbm, wo_hbm, w1_hbm, b1_hbm, w2_hbm, b2_hbm, out_ref,
             kb32, vb32, wq32, wo32, kring, vring, w1b, w2b, xb, b1b, b2b,
             x_s, xn_s, q_s, s_s, p_s, a_s, o_s, acc_s, zero_s,
             semk, semv, semw):
        def slab_copies(m):
            rows, slot = _ds(m * LANES, LANES, LANES), m % RING
            return [_Copy(src.at[rows, pl.ds(SK - W, W)], ring.at[slot], sem.at[slot], SPL)
                    for src, ring, sem in ((v_hbm, vring, semv), (k_hbm, kring, semk))]

        def wq_copy(c):
            return _Copy(wq_hbm.at[:, _ds(c * F, F, LANES)], w1b, semw.at[0], SPW)

        def wo_copy(i, n, staged):
            return _Copy(
                wo_hbm.at[_ds(i * PAIR, n * PAIR, PAIR)], w2b.at[pl.ds(staged * PAIR, n * PAIR)],
                semw.at[1 + staged // U], SPW)

        w1_copy = _Copy(w1_hbm, w1b, semw.at[0], SPW)
        w2_rows = [pl.ds(n * F // NW, F // NW) for n in range(NW)]
        w2_copies = [_Copy(w2_hbm.at[r], w2b.at[r], semw.at[6 + n], SPW // NW)
                     for n, r in enumerate(w2_rows)]
        small = [pltpu.make_async_copy(s, d, semw.at[3 + n])
                 for n, (s, d) in enumerate(((x_hbm, xb), (b1_hbm, b1b), (b2_hbm, b2b)))]

        def pack_wq(c):
            wq_copy(c).wait()

            @pl.loop(0, NF)
            def _(j):
                wq32[c * NF + j] = pltpu.bitcast(w1b[:, _ds(j * LANES, LANES, LANES)], u32)

        def pack_wo(i, staged):
            @pl.loop(0, ND)
            def _(j):
                w = w2b[_ds(staged * PAIR, PAIR, PAIR), _ds(j * LANES, LANES, LANES)]
                wo32[j, _ds(i * DH, DH, 8), :] = pltpu.bitcast(w, u32)

        def pack_slab(m):
            def pack(dst, ring, lo, hi, step, transpose=False):
                @pl.loop(lo, hi)
                def _(g):
                    for j in range(step):
                        t = ring[m % RING, :, _ds((g * step + j) * LANES, LANES, LANES)]
                        dst[g * step + j, _ds(m * (LANES // 2), LANES // 2, 8), :] = pltpu.bitcast(
                            t.T if transpose else t, u32)

            v_copy, k_copy = slab_copies(m)
            last = m >= NSLAB - 3
            v_copy.wait()
            pack(vb32, vring, 0, jnp.where(last, NML // NM, 1), NM, True)
            pack(vb32, vring, jnp.where(last, NML // 2, NM // 2), NS // 2, 2)
            k_copy.wait()
            pack(kb32, kring, 0, NC, 4)

            @pl.when(m + RING < NSLAB)
            def _():
                for c in slab_copies(m + RING):
                    c.start()

            @pl.when(m + RING == NSLAB - 1)
            def _():
                for c in [w1_copy] + w2_copies:
                    c.start()

        def fetch(b):
            wo_copy(b * U, U, 0).wait()
            pl.loop(0, U)(lambda u: pack_wo(b * U + u, u))
            pl.when(b + 1 < NB)(lambda: wo_copy((b + 1) * U, U, 0).start())

            @pl.when(b + 1 < NQ)
            def _():
                pack_wq(b + 1)
                pl.when(b + 2 < NQ)(lambda: wq_copy(b + 2).start())

            pl.loop(3 * (b * U + 1), 3 * (b * U + 1 + U))(pack_slab)

        for m in range(RING):
            for c in slab_copies(m):
                c.start()
        for c in small + [wq_copy(0), wo_copy(0, U, 0), wo_copy(NP - 1, 1, U)]:
            c.start()
        zero_s[...] = jnp.zeros((8, LANES), jnp.int32)
        pl.loop(0, 3)(pack_slab)
        for c in small:
            c.wait()
        x_s[...] = jnp.broadcast_to(xb[0].astype(f32), (8, D))
        pack_wq(0)
        wq_copy(1).start()
        wo_copy(NP - 1, 1, U).wait()
        pack_wo(NP - 1, U)

        row = _iota((8, LANES), 0)
        upper = (_iota((8, LANES), 1) >= DH - LANES).astype(jnp.int32)
        head_of_lane = [(n + upper) >> 1 for n in range(3)]
        own_head = jnp.concatenate([(row & 1) - h for h in head_of_lane], axis=1) == 0

        def q_proj(i):
            return _dot(xn_s[...], _tiles(wq32, 3 * i, 3, 0, D))

        def q_blocks(q):
            q = _round(q)
            return jnp.concatenate(
                [jnp.where(row == 2 * t + head_of_lane[n], _lane_tile(q, n), 0.0)
                 for n in range(3) for t in range(4)], axis=1)

        def scores(q, i, mark=lambda v, cost: v):
            cols = []
            for c in range(NC):
                y = None
                for n in range(3):
                    k = jnp.concatenate(
                        [_tile(kb32, 4 * c + t, i * PAIR + n * LANES, LANES) for t in range(4)], axis=0)
                    z = _dot(q[:, 4 * n * LANES:4 * (n + 1) * LANES], k)
                    y = mark(z if y is None else y + z, 4)
                cols.append(y)
            return jnp.concatenate(cols, axis=1)

        def per_head(v, op):
            v = jnp.broadcast_to(v, (8, LANES))
            v = op(v, pltpu.roll(v, 2, 0))
            return op(v, pltpu.roll(v, 4, 0))

        def softmax(s):
            m = per_head(jnp.max(s, axis=1, keepdims=True), jnp.maximum)
            e = jnp.exp2((s - jnp.concatenate([m] * NC, axis=1)) * exp_scale)
            return e, per_head(jnp.sum(e, axis=1, keepdims=True), jnp.add)

        def pv_mxu(i, e, nm):
            p = jnp.concatenate(
                [jnp.where((row >> 1) == j % 4, _lane_tile(e, j // 4), 0.0) for j in range(nm)], axis=1)
            v = jnp.concatenate(
                [jnp.concatenate([_tile(vb32, j, i * PAIR + n * LANES, LANES) for j in range(nm)], axis=0)
                 for n in range(3)], axis=1)
            return _dot(p, v)

        def pv_vpu(i, u, g, nm, never, after):
            a = g * VROWS // DH
            acc = None
            for j in range(nm, NS):
                c, t = divmod(j, 4)
                p = jnp.broadcast_to(p_s[u, 2 * t + a:2 * t + a + 1, c * LANES:(c + 1) * LANES], (8, LANES))
                seg, off = divmod(j - nm, pl.cdiv(NS - nm, NT))
                if off == 0 and after[seg] is not None:
                    p = jnp.where(never, after[seg], p)
                v = _tile(vb32, j, i * PAIR + g * VROWS, VROWS).astype(f32)
                y = v * jnp.concatenate([p] * (VROWS // 8), axis=0)
                acc = y if acc is None else acc + y
            return acc

        def head_out(a, om, ol):
            o = jnp.sum(jnp.concatenate([a.T, om], axis=0), axis=0, keepdims=True)
            return jnp.broadcast_to(o / jnp.sum(ol, axis=0, keepdims=True), (8, PAIR))

        def o_proj(o, i):
            return _dot(o, _tiles(wo32, 0, ND, i * PAIR, PAIR))

        def attend(i0, n, last):
            nm = NML if last else NM
            never = zero_s[...] != 0
            marks = []

            def mark(v, tiles):
                for m in range(v.shape[1] // LANES):
                    marks.append(((marks[-1][0] if marks else 0) + 8 * tiles, _lane_tile(v, m)))
                return v

            s, q, a, om, ol, acc = s_s[...], q_s[...], a_s[...], o_s[0], o_s[1], acc_s[...]
            ng = PAIR // VROWS
            span = n * 8 * (3 * NS + 6 * ND + 3 * nm) - 60
            for u in range(n):
                i = i0 + u
                e, l = softmax(s)
                p_s[u] = e
                o_prev = head_out(a, om, ol)
                if not last:
                    s = scores(q, i + 1, mark)
                om = jnp.where(own_head, mark(pv_mxu(i, e, nm), nm), 0.0)
                ol = jnp.where(own_head, jnp.concatenate([l * 0.25] * 3, axis=1), 0.0)
                if not last:
                    q = q_blocks(mark(q_proj(jnp.minimum(i + 2, NP - 1)), ND))
                acc = acc + mark(o_proj(o_prev, jnp.maximum(i - 1, 0)), 3)
                parts = []
                for g in range(ng):
                    ready = [0] + [sum(t <= (u * ng + g + seg / NT) * span / (n * ng) for t, _ in marks)
                                   for seg in range(NT)]
                    after = [marks[r - 1][1] if r > r0 and not last else None
                             for r0, r in zip(ready, ready[1:])]
                    parts.append(pv_vpu(i, u, g, nm, never, after))
                a = jnp.concatenate(parts, axis=0)
            if last:
                return acc + o_proj(head_out(a, om, ol), i0)
            s_s[...], q_s[...], a_s[...], o_s[0], o_s[1], acc_s[...] = s, q, a, om, ol, acc

        @pl.loop(0, 2)
        def _(layer):
            first = layer == 0
            xn_s[...] = _layernorm(x_s[...])
            q0, q_s[...] = q_blocks(q_proj(0)), q_blocks(q_proj(1))
            s_s[...] = scores(q0, 0)
            a_s[...] = jnp.zeros((PAIR, LANES), f32)
            o_s[0] = jnp.zeros((8, PAIR), f32)
            o_s[1] = jnp.ones((8, PAIR), f32)
            acc_s[...] = jnp.zeros((8, D), f32)

            @pl.loop(0, NB)
            def _(b):
                pl.when(first)(lambda: fetch(b))
                attend(b * U, U, False)

            x = _round(x_s[...] + _round(attend(NP - 1, 1, True)))
            xn = _layernorm(x)

            def mlp(arriving):
                if arriving:
                    w1_copy.wait()
                h = _round(_round(_dot(xn, w1b[...])) + b1b[...].astype(f32).reshape(1, F))
                h = jax.nn.gelu(h, approximate=True)
                if arriving:
                    y = 0.0
                    for c, r in zip(w2_copies, w2_rows):
                        c.wait()
                        y = y + _dot(h[:, r.start:r.start + r.size], w2b[r, :])
                else:
                    y = _dot(h, w2b[...])
                x_s[...] = _round(x + _round(_round(y) + b2b[...].astype(f32).reshape(1, D)))

            pl.when(first)(lambda: mlp(True))
            pl.when(layer != 0)(lambda: mlp(False))

        out_ref[0] = x_s[0:1, :].astype(out_ref.dtype)

    vmem, dma = pltpu.VMEM, pltpu.SemaphoreType.DMA
    return pl.pallas_call(
        body,
        out_shape=jax.ShapeDtypeStruct((1, 1, D), bf16),
        in_specs=[pl.BlockSpec(memory_space=pl.ANY)] * 9,
        scratch_shapes=[
            vmem((NS, H * DH // 2 + 8, LANES), u32), vmem((NS, H * DH // 2 + 24, LANES), u32),
            vmem((NSLAB, D // 2, LANES), u32), vmem((ND, H * DH // 2, LANES), u32),
            vmem((RING, LANES, W), bf16), vmem((RING, LANES, W), bf16),
            vmem((D, F), bf16), vmem((F, D), bf16),
            vmem((1, 1, D), bf16), vmem((F,), bf16), vmem((D,), bf16),
            vmem((8, D), f32), vmem((8, D), f32), vmem((8, 4 * PAIR), f32), vmem((8, W // 4), f32),
            vmem((U, 8, W // 4), f32), vmem((PAIR, LANES), f32), vmem((2, 8, PAIR), f32),
            vmem((8, D), f32), vmem((8, LANES), jnp.int32),
            dma((RING,)), dma((RING,)), dma((6 + NW,)),
        ],
        compiler_params=pltpu.CompilerParams(vmem_limit_bytes=124 * 1024 * 1024),
        name="fused_layers",
    )


@jax.jit
def pallas_interleave_layers__sliding_block_cached__dense_activation_gelu__decode_kernel(
    A_x: jax.Array,
    A_k_cache: jax.Array,
    A_v_cache: jax.Array,
    A_wq: jax.Array,
    A_wo: jax.Array,
    B_x: jax.Array,
    B_w1: jax.Array,
    B_b1: jax.Array,
    B_w2: jax.Array,
    B_b2: jax.Array,
):
    del B_x
    SK = A_k_cache.shape[2]
    W = min(4096, max(256, SK // 4))
    D, F = B_w1.shape
    kt = jnp.swapaxes(A_k_cache, 2, 3).reshape(H * DH, SK)
    vt = jnp.swapaxes(A_v_cache, 2, 3).reshape(H * DH, SK)
    return _build(SK, W, D, F)(A_x, kt, vt, A_wq, A_wo, B_w1, B_b1, B_w2, B_b2)
```
